```python
import jax
import jax.numpy as jnp

def _softmax(x, axis=-1):
    return jax.nn.softmax(x, axis=axis)

def _gelu(x):
    return jax.nn.gelu(x, approximate=True)

def _silu(x):
    return jax.nn.silu(x)

def _sigmoid(x):
    return jax.nn.sigmoid(x)

def _layernorm(x, axis=-1, eps=1e-05):
    m = jnp.mean(x, axis=axis, keepdims=True)
    v = jnp.var(x, axis=axis, keepdims=True)
    return (x - m) / jnp.sqrt(v + eps)

def _scatter_add(tgt, idx, src, axis=0):
    return tgt.at[idx].add(src)

def _segment_sum(src, seg, n):
    return jax.ops.segment_sum(src, seg, n)

class _Rng:

    def __init__(self, key):
        self._k = key

    def _next(self):
        self._k, sub = jax.random.split(self._k)
        return sub

    def normal(self, shape):
        return jax.random.normal(self._next(), shape, dtype=jnp.bfloat16)

    def randint(self, lo, hi, shape):
        return jax.random.randint(self._next(), shape, lo, hi, dtype=jnp.int32)

    def uniform(self, shape, lo=0.0, hi=1.0):
        return jax.random.uniform(self._next(), shape, jnp.bfloat16, lo, hi)

    def permutation(self, n):
        return jax.random.permutation(self._next(), n)
kernel_name = 'adaLN_cond__sliding_block_cached__mixer_channel_mlp__decode'

def setup_inputs():
    _rng = _Rng(jax.random.key(int.from_bytes(__import__("os").urandom(4), "little")))
    _w = lambda a: (lambda t: t.astype(jnp.bfloat16) if jnp.issubdtype(t.dtype, jnp.floating) else t)(jnp.asarray(a))

    def _A_setup():
        B, Sq, D = (8, 1, 640)
        Hq, Hkv, Sk, Dh = (32, 32, 4096, 192)
        assert Hq % Hkv == 0, (Hq, Hkv)
        return {'x': _w((lambda *s: _rng.normal(s) * 0.05)(B, Sq, D)), 'k_cache': _w((lambda *s: _rng.normal(s) * 0.05)(B, Hkv, Sk, Dh)), 'v_cache': _w((lambda *s: _rng.normal(s) * 0.05)(B, Hkv, Sk, Dh)), 'wq': _w((lambda *s: _rng.normal(s) * 0.05)(D, Hq * Dh) * D ** (-0.5)), 'wo': _w((lambda *s: _rng.normal(s) * 0.05)(Hq * Dh, D) * (Hq * Dh) ** (-0.5))}
    _A_in = _A_setup()

    def _B_setup():
        B, S, D, F = (8, 1, 640, 1536)
        return {'x': _w((lambda *s: _rng.normal(s) * 0.05)(B, S, D)), 'w1': _w((lambda *s: _rng.normal(s) * 0.05)(D, F) * D ** (-0.5)), 'b1': _w((lambda *s: _rng.normal(s) * 0.05)(F)), 'w2': _w((lambda *s: _rng.normal(s) * 0.05)(F, D) * F ** (-0.5)), 'b2': _w((lambda *s: _rng.normal(s) * 0.05)(D))}
    _B_in = _B_setup()
    return {'A_x': _A_in['x'], 'A_k_cache': _A_in['k_cache'], 'A_v_cache': _A_in['v_cache'], 'A_wq': _A_in['wq'], 'A_wo': _A_in['wo'], 'B_x': _B_in['x'], 'B_w1': _B_in['w1'], 'B_b1': _B_in['b1'], 'B_w2': _B_in['w2'], 'B_b2': _B_in['b2'], 'c': _w((lambda *s: _rng.normal(s) * 0.05)(8, 640)), 'w_mod': _w((lambda *s: _rng.normal(s) * 0.05)(640, 6 * 640) * 640 ** (-0.5))}

def reference(A_x, A_k_cache, A_v_cache, A_wq, A_wo, B_x, B_w1, B_b1, B_w2, B_b2, c, w_mod):

    def _A_ref(x, k_cache, v_cache, wq, wo):
        B, Sq, D = x.shape
        Hq, Dh = (32, 192)
        Hkv, Sk = (k_cache.shape[1], k_cache.shape[2])
        W = min(4096, max(256, Sk // 4))
        rep = Hq // Hkv
        q = (lambda x, *d: x.transpose(*d))((x @ wq).reshape(B, Sq, Hq, Dh), 0, 2, 1, 3)
        k = jnp.repeat(k_cache[:, :, Sk - W:, :], rep, axis=1)
        v = jnp.repeat(v_cache[:, :, Sk - W:, :], rep, axis=1)
        scores = jnp.einsum('bhqd,bhkd->bhqk', q, k) * Dh ** (-0.5)
        p = _softmax(scores, axis=-1)
        o = jnp.einsum('bhqk,bhkd->bhqd', p, v)
        return (lambda x, *d: x.transpose(*d))(o, 0, 2, 1, 3).reshape(B, Sq, Hq * Dh) @ wo

    def _B_ref(x, w1, b1, w2, b2):
        y = _layernorm(x, axis=-1)
        h = _gelu(jnp.einsum('bsd,df->bsf', y, w1) + b1)
        return jnp.einsum('bsf,fd->bsd', h, w2) + b2
    x = A_x
    mod = (_silu(c) @ w_mod).reshape(c.shape[0], 6, 1, -1)
    sa, ca, ga, sb, cb, gb = (mod[:, 0].copy(), mod[:, 1].copy(), mod[:, 2].copy(), mod[:, 3].copy(), mod[:, 4].copy(), mod[:, 5].copy())
    h = _layernorm(x, axis=-1) * (1 + ca) + sa
    x = x + ga * _A_ref(h, A_k_cache, A_v_cache, A_wq, A_wo)
    h = _layernorm(x, axis=-1) * (1 + cb) + sb
    x = x + gb * _B_ref(h, B_w1, B_b1, B_w2, B_b2)
    return x
```

```python
import jax
import jax.numpy as jnp
from jax import lax
from jax.experimental import pallas as pl
from jax.experimental.pallas import tpu as pltpu

_EPS = 1e-05
_G = 8
_NBUF = 4
_WQ_CHUNKS = 4
_WO_CHUNKS = 4
_W2_CHUNKS = 4


def _layernorm(x):
    m = jnp.mean(x, axis=-1, keepdims=True)
    d = x - m
    v = jnp.mean(d * d, axis=-1, keepdims=True)
    return d / jnp.sqrt(v + _EPS)


def _kernel(x_hbm, k_hbm, v_hbm, wq_hbm, wo_hbm, w1_hbm, b1_hbm, w2_hbm, b2_hbm, c_hbm, wmod_hbm,
            out_ref,
            x_v, c_v, b1_v, b2_v, wmod_v, wq_v, wo_v, w1_v, w2_v, k_v, v_v, q_s, o_s, mod_s,
            sem_misc, sem_wq, sem_wo, sem_w2, sem_k, sem_v):
    B, D = x_v.shape
    HD = wq_v.shape[1]
    F = w1_v.shape[1]
    SK = k_hbm.shape[2]
    nbuf, GD, W = k_v.shape
    Dh = GD // _G
    NG = HD // GD
    nsteps = B * NG

    def kv_copies(i, slot):
        b = i % B
        g = i // B
        rows = pl.ds(pl.multiple_of(g * GD, GD), GD)
        cols = pl.ds(SK - W, W)
        return (pltpu.make_async_copy(k_hbm.at[b, rows, cols], k_v.at[slot], sem_k.at[slot]),
                pltpu.make_async_copy(v_hbm.at[b, rows, cols], v_v.at[slot], sem_v.at[slot]))

    cp_wmod = pltpu.make_async_copy(wmod_hbm, wmod_v, sem_misc.at[0])
    cp_c = pltpu.make_async_copy(c_hbm, c_v, sem_misc.at[1])
    cp_x = pltpu.make_async_copy(x_hbm, x_v, sem_misc.at[2])
    cp_b1 = pltpu.make_async_copy(b1_hbm, b1_v, sem_misc.at[3])
    cp_b2 = pltpu.make_async_copy(b2_hbm, b2_v, sem_misc.at[4])
    cp_w1 = pltpu.make_async_copy(w1_hbm, w1_v, sem_misc.at[5])
    qc = HD // _WQ_CHUNKS
    cp_wq = [pltpu.make_async_copy(wq_hbm.at[:, pl.ds(j * qc, qc)], wq_v.at[:, pl.ds(j * qc, qc)], sem_wq.at[j])
             for j in range(_WQ_CHUNKS)]
    oc = HD // _WO_CHUNKS
    cp_wo = [pltpu.make_async_copy(wo_hbm.at[pl.ds(j * oc, oc)], wo_v.at[pl.ds(j * oc, oc)], sem_wo.at[j])
             for j in range(_WO_CHUNKS)]
    fc = F // _W2_CHUNKS
    cp_w2 = [pltpu.make_async_copy(w2_hbm.at[pl.ds(j * fc, fc)], w2_v.at[pl.ds(j * fc, fc)], sem_w2.at[j])
             for j in range(_W2_CHUNKS)]

    cp_wmod.start()
    cp_c.start()
    cp_wq[0].start()
    cp_x.start()
    for j in range(1, _WQ_CHUNKS):
        cp_wq[j].start()
    for i in range(nbuf):
        ck, cv = kv_copies(i, i)
        ck.start()
        if i == 0:
            cp_b1.start()
        cv.start()
        if i == 0:
            cp_b2.start()

    cp_wmod.wait()
    cp_c.wait()
    cf = c_v[...].astype(jnp.float32)
    sc = (cf * jax.nn.sigmoid(cf)).astype(jnp.bfloat16)
    mod_s[...] = jnp.dot(sc, wmod_v[...], preferred_element_type=jnp.float32)
    cp_x.wait()
    xf = x_v[...].astype(jnp.float32)
    h = (_layernorm(xf) * (1.0 + mod_s[:, D:2 * D]) + mod_s[:, 0:D]).astype(jnp.bfloat16)
    per = _WQ_CHUNKS // NG
    for g in range(NG):
        for j in range(per):
            cp_wq[g * per + j].wait()
        q_s[g] = jnp.dot(h, wq_v[:, g * GD:(g + 1) * GD], preferred_element_type=jnp.float32)

    row = lax.broadcasted_iota(jnp.int32, (_G, GD), 0)
    col = lax.broadcasted_iota(jnp.int32, (_G, GD), 1)
    diag = jnp.logical_and(col >= row * Dh, col < (row + 1) * Dh)
    scale = Dh ** -0.5

    def step(i, slot, after_k=None, after_v=None):
        b = i % B
        g = i // B
        ck, cv = kv_copies(i, slot)
        qrow = q_s[g, pl.ds(b, 1), :]
        qbd = jnp.where(diag, jnp.broadcast_to(qrow, (_G, GD)), 0.0).astype(jnp.bfloat16)
        ck.wait()
        s = jnp.dot(qbd, k_v[slot], preferred_element_type=jnp.float32) * scale
        if after_k is not None:
            after_k()
        m = jnp.max(s, axis=-1, keepdims=True)
        p = jnp.exp(s - m)
        l = jnp.sum(p, axis=-1, keepdims=True)
        cv.wait()
        o = lax.dot_general(p.astype(jnp.bfloat16), v_v[slot], (((1,), (1,)), ((), ())),
                            preferred_element_type=jnp.float32)
        if after_v is not None:
            after_v()
        o = jnp.where(diag, o / l, 0.0)
        o_s[g, pl.ds(b, 1), :] = jnp.sum(o, axis=0, keepdims=True)

    def body(i, carry):
        slot = i % nbuf
        nk, nv = kv_copies(i + nbuf, slot)
        step(i, slot, nk.start, nv.start)
        return carry

    lax.fori_loop(0, nsteps - nbuf, body, 0)

    for cp in cp_wo:
        cp.start()
    cp_w1.start()
    for cp in cp_w2:
        cp.start()

    def body2(i, carry):
        step(i, i % nbuf)
        return carry

    lax.fori_loop(nsteps - nbuf, nsteps, body2, 0)

    attn = None
    per = _WO_CHUNKS // NG
    for g in range(NG):
        for j in range(per):
            cp_wo[g * per + j].wait()
        part = jnp.dot(o_s[g].astype(jnp.bfloat16), wo_v[g * GD:(g + 1) * GD, :],
                       preferred_element_type=jnp.float32)
        attn = part if attn is None else attn + part
    x1 = xf + mod_s[:, 2 * D:3 * D] * attn
    h2 = _layernorm(x1) * (1.0 + mod_s[:, 4 * D:5 * D]) + mod_s[:, 3 * D:4 * D]
    y = _layernorm(h2).astype(jnp.bfloat16)
    cp_b1.wait()
    cp_b2.wait()
    b1 = b1_v[...].astype(jnp.float32).reshape(1, F)
    b2 = b2_v[...].astype(jnp.float32).reshape(1, D)
    cp_w1.wait()
    u = jnp.dot(y, w1_v[...], preferred_element_type=jnp.float32) + b1
    a = jax.nn.gelu(u, approximate=True).astype(jnp.bfloat16)
    acc = jnp.broadcast_to(b2, (B, D))
    for j in range(_W2_CHUNKS):
        cp_w2[j].wait()
        acc = acc + jnp.dot(a[:, j * fc:(j + 1) * fc], w2_v[j * fc:(j + 1) * fc, :],
                            preferred_element_type=jnp.float32)
    out_ref[...] = (x1 + mod_s[:, 5 * D:6 * D] * acc).astype(out_ref.dtype)


@jax.jit
def pallas_adaLN_cond__sliding_block_cached__mixer_channel_mlp__decode_kernel(
    A_x: jax.Array,
    A_k_cache: jax.Array,
    A_v_cache: jax.Array,
    A_wq: jax.Array,
    A_wo: jax.Array,
    B_x: jax.Array,
    B_w1: jax.Array,
    B_b1: jax.Array,
    B_w2: jax.Array,
    B_b2: jax.Array,
    c: jax.Array,
    w_mod: jax.Array,
):
    del B_x
    B, Sq, D = A_x.shape
    _, Hkv, SK, Dh = A_k_cache.shape
    W = min(4096, max(256, SK // 4))
    HD = A_wq.shape[1]
    F = B_w1.shape[1]
    GD = _G * Dh
    kt = jnp.swapaxes(A_k_cache, 2, 3).reshape(B, Hkv * Dh, SK)
    vt = jnp.swapaxes(A_v_cache, 2, 3).reshape(B, Hkv * Dh, SK)
    bf = jnp.bfloat16
    f32 = jnp.float32
    dma = pltpu.SemaphoreType.DMA
    out = pl.pallas_call(
        _kernel,
        out_shape=jax.ShapeDtypeStruct((B, D), A_x.dtype),
        in_specs=[pl.BlockSpec(memory_space=pltpu.HBM)] * 11,
        out_specs=pl.BlockSpec(memory_space=pltpu.VMEM),
        scratch_shapes=[
            pltpu.VMEM((B, D), bf), pltpu.VMEM((B, D), bf), pltpu.VMEM((F,), bf), pltpu.VMEM((D,), bf),
            pltpu.VMEM((D, 6 * D), bf), pltpu.VMEM((D, HD), bf), pltpu.VMEM((HD, D), bf),
            pltpu.VMEM((D, F), bf), pltpu.VMEM((F, D), bf),
            pltpu.VMEM((_NBUF, GD, W), bf), pltpu.VMEM((_NBUF, GD, W), bf),
            pltpu.VMEM((HD // GD, B, GD), f32), pltpu.VMEM((HD // GD, B, GD), f32),
            pltpu.VMEM((B, 6 * D), f32),
            dma((6,)), dma((_WQ_CHUNKS,)), dma((_WO_CHUNKS,)), dma((_W2_CHUNKS,)),
            dma((_NBUF,)), dma((_NBUF,)),
        ],
        compiler_params=pltpu.CompilerParams(vmem_limit_bytes=100 * 1024 * 1024),
    )(A_x.reshape(B, D), kt, vt, A_wq, A_wo, B_w1, B_b1, B_w2, B_b2, c, w_mod)
    return out.reshape(B, Sq, D)
```

```python
import functools

import jax
import jax.numpy as jnp
from jax import lax
from jax.experimental import pallas as pl
from jax.experimental.pallas import tpu as pltpu

_EPS = 1e-05
bf = jnp.bfloat16
f32 = jnp.float32


def _layernorm(x):
    m = jnp.mean(x, axis=-1, keepdims=True)
    d = x - m
    v = jnp.mean(d * d, axis=-1, keepdims=True)
    return d / jnp.sqrt(v + _EPS)


def make(compute=True, n0=1, p_small=0, p_big=1, wq0=1024, wo0=16, checks=False, schecks=False, CW=512, bunch=False):
    G = 8
    NB = 4
    NSLOT = 3

    def kernel(x_hbm, k_hbm, v_hbm, wq_hbm, wo_hbm, w1_hbm, b1_hbm, w2_hbm, b2_hbm, c_hbm, wmod_hbm,
               out_ref,
               x_v, c_v, b1_v, b2_v, wmod_v, wq_v, wo_v, w1_v, w2_v, k_v, v_v, q_s, o_s, mod_s,
               sem_misc, sem_w, sem_kv):
        B, D = x_v.shape
        F = w1_v.shape[1]
        _, _, S, _, W = k_v.shape
        SK = k_hbm.shape[-1]
        NG = k_hbm.shape[1]
        BR = S * 8
        Dh = BR // 2
        nsteps = B * NG
        NI = 2 * NB
        M = S // NI
        scale = Dh ** -0.5
        win = pl.ds(SK - W, W)

        class Ev:
            def __init__(self, small, big):
                self.small, self.big = small, big

            def start(self):
                if self.small is not None:
                    self.small.start(priority=p_small)
                self.big.start(priority=p_big)

        def kv_event(step, it, e):
            slot = step % NSLOT
            b = step % B
            g = step // B
            src, dst = ((k_hbm, k_v), (v_hbm, v_v))[e % 2]
            pos = (e // 2) * NI + it
            return Ev(
                pltpu.make_async_copy(src.at[b, g, pl.ds(0, n0), pos, :, win],
                                      dst.at[slot, pl.ds(0, n0), pos], sem_kv.at[0, slot]),
                pltpu.make_async_copy(src.at[b, g, pl.ds(n0, NB - n0), pos, :, win],
                                      dst.at[slot, pl.ds(n0, NB - n0), pos], sem_kv.at[1, slot]))

        def kv_wait_small(step):
            slot = step % NSLOT
            for dst in (k_v, v_v):
                d = dst.at[slot, pl.ds(0, n0)]
                pltpu.make_async_copy(d, d, sem_kv.at[0, slot]).wait()

        def rows(i, n):
            return pl.ds(pl.multiple_of(i * n, n), n)

        def wmod_event(i):
            return Ev(None, pltpu.make_async_copy(wmod_hbm.at[rows(i, 8)], wmod_v.at[rows(i, 8)], sem_w.at[0]))

        def wq_event(i):
            lo, hi = pl.ds(0, wq0), pl.ds(wq0, wq_v.shape[1] - wq0)
            return Ev(pltpu.make_async_copy(wq_hbm.at[rows(i, 8), lo], wq_v.at[rows(i, 8), lo], sem_w.at[1]),
                      pltpu.make_async_copy(wq_hbm.at[rows(i, 8), hi], wq_v.at[rows(i, 8), hi], sem_w.at[2]))

        def row_event(src, dst, i, n, n_small, s_small, s_big):
            lo = pl.ds(pl.multiple_of(i * n, 8), n_small)
            hi = pl.ds(pl.multiple_of(i * n + n_small, 8), n - n_small)
            return Ev(pltpu.make_async_copy(src.at[lo], dst.at[lo], sem_w.at[s_small]),
                      pltpu.make_async_copy(src.at[hi], dst.at[hi], sem_w.at[s_big]))

        def wo_event(i):
            return row_event(wo_hbm, wo_v, i, 64, wo0, 3, 4)

        def w1_event(i):
            return row_event(w1_hbm, w1_v, i, 40, 8, 5, 6)

        def w2_event(i, j):
            return row_event(w2_hbm, w2_v, i * 6 + j, 64, wo0, 7 + 2 * i, 8 + 2 * i)

        cp_c = pltpu.make_async_copy(c_hbm, c_v, sem_misc.at[0])
        cp_x = pltpu.make_async_copy(x_hbm, x_v, sem_misc.at[1])
        cp_b1 = pltpu.make_async_copy(b1_hbm, b1_v, sem_misc.at[2])
        cp_b2 = pltpu.make_async_copy(b2_hbm, b2_v, sem_misc.at[3])

        def loop(n, body, init=0):
            return lax.fori_loop(0, n, body, init)

        def ph0(i, c):
            wmod_event(i).start()
            return c
        loop(D // 8, ph0)
        for cp in (cp_c, cp_x, cp_b1, cp_b2):
            cp.start(priority=p_small)

        def ph1(i, c):
            wmod_event(i).big.wait()
            wq_event(i).start()
            return c
        loop(D // 8, ph1)
        for cp in (cp_c, cp_x, cp_b1, cp_b2):
            cp.wait()

        cf = c_v[...].astype(f32)
        sc = (cf * jax.nn.sigmoid(cf)).astype(bf)

        def ph2(it, c):
            for e in range(2 * M):
                if e < 10:
                    wq_event(it * 10 + e).big.wait()
                kv_event(0, it, e).start()
            return c
        loop(NI, ph2)
        if compute:
            def modj(j, c):
                mod_s[j] = jnp.dot(sc, wmod_v[:, pl.ds(pl.multiple_of(j * D, 128), D)], preferred_element_type=f32)
                return c
            loop(6, modj)

        def wq_small_wait(i, c):
            wq_event(i).small.wait()
            return c
        loop(D // 8, wq_small_wait)

        xf = x_v[...].astype(f32)
        h = (_layernorm(xf) * (1.0 + mod_s[1]) + mod_s[0]).astype(bf)

        def ph3(it, c):
            for half in range(2):
                hp = it * 2 + half
                for t in range(3):
                    for e in range(2):
                        ee = half * M + t * 2 + e
                        kv_event(0, it, ee).big.wait()
                        kv_event(1, it, ee).start()
                    if compute:
                        col = pl.ds(pl.multiple_of(hp * BR + t * 128, 128), 128)
                        q_s[hp, :, t * 128:(t + 1) * 128] = jnp.dot(h, wq_v[:, col], preferred_element_type=f32)
            return c
        loop(NI, ph3)
        kv_wait_small(0)

        row = lax.broadcasted_iota(jnp.int32, (G, BR), 0)
        hi_half = (lax.broadcasted_iota(jnp.int32, (G, BR), 1) >= Dh).astype(jnp.int32)

        def attention(step, pump):
            slot = step % NSLOT
            b = step % B
            g = step // B

            def qk(it, s):
                if compute:
                    qrow = q_s[g * NB + it, pl.ds(b, 1), :]
                    qbd = jnp.where(row == 2 * it + hi_half, jnp.broadcast_to(qrow, (G, BR)), 0.0).astype(bf)
                parts = []
                NP = CW // 256
                for n in range(W // CW):
                    acc = None
                    for t in range(3):
                        e0 = (n * 3 + t) * NP
                        pre = NP if bunch else (NP + 1) // 2
                        pump(it, range(e0, e0 + pre))
                        if compute:
                            kt = k_v[slot, it, pl.ds(t * 16, 16), :, pl.ds(n * CW, CW)].reshape(128, CW)
                            d = jnp.dot(qbd[:, t * 128:(t + 1) * 128], kt, preferred_element_type=f32)
                            acc = d if acc is None else acc + d
                        pump(it, range(e0 + pre, e0 + NP))
                    parts.append(acc)
                if compute:
                    s = s + jnp.concatenate(parts, axis=1)
                return s
            s = loop(NB, qk, jnp.zeros((G, W), f32)) * scale
            m = jnp.max(s, axis=-1, keepdims=True)
            p = jnp.exp(s - m)
            inv = 1.0 / jnp.sum(p, axis=-1, keepdims=True)
            pb = p.astype(bf)

            def pv(it, c):
                parts = []
                NP = CW // 256
                for t in range(3):
                    acc = None
                    for n in range(W // CW):
                        e0 = (t * (W // CW) + n) * NP
                        pre = NP if bunch else (NP + 1) // 2
                        pump(NB + it, range(e0, e0 + pre))
                        if compute:
                            vt = v_v[slot, it, pl.ds(t * 16, 16), :, pl.ds(n * CW, CW)].reshape(128, CW)
                            d = lax.dot_general(pb[:, n * CW:(n + 1) * CW], vt, (((1,), (1,)), ((), ())),
                                                preferred_element_type=f32)
                            acc = d if acc is None else acc + d
                        pump(NB + it, range(e0 + pre, e0 + NP))
                    parts.append(acc)
                if compute:
                    o = jnp.concatenate(parts, axis=1) * inv
                    o = jnp.where(row == 2 * it + hi_half, o, 0.0)
                    o_s[g * NB + it, pl.ds(b, 1), :] = jnp.sum(o, axis=0, keepdims=True)
                return c
            loop(NB, pv)

        def ph4(s, c):
            def pump(it, es):
                for e in es:
                    kv_event(s, it, e).big.wait()
                for e in es:
                    kv_event(s + 1, it, e).start()
            attention(s - 1, pump)
            kv_wait_small(s)
            return c
        lax.fori_loop(1, nsteps - 1, ph4, 0)

        def pump5(it, es):
            for e in es:
                kv_event(nsteps - 1, it, e).big.wait()
            for e in es:
                wo_event(it * 2 * M + e).start()
        attention(nsteps - 2, pump5)
        kv_wait_small(nsteps - 1)

        def pump6(it, es):
            for e in es:
                wo_event(it * 2 * M + e).big.wait()
                if e % 6 == 0:
                    w1_event(it * 2 + e // 6).start()
        attention(nsteps - 1, pump6)

        def wo_small_wait(i, c):
            wo_event(i).small.wait()
            return c
        loop(96, wo_small_wait)

        def ph7(i, acc):
            for j in range(4):
                w1_event(i * 4 + j).big.wait()
                if j < 3:
                    w2_event_dyn(i, 2 * j).start()
                    w2_event_dyn(i, 2 * j + 1).start()
                if compute:
                    hp = i * 4 + j
                    acc = acc + jnp.dot(o_s[hp].astype(bf), wo_v[rows(hp, BR), :], preferred_element_type=f32)
            return acc

        def w2_event_dyn(i, j):
            return w2_event(i, j)
        attn = jnp.zeros((B, D), f32)
        for i in range(4):
            attn = ph7(i, attn)

        def w1_small_wait(i, c):
            w1_event(i).small.wait()
            return c
        loop(16, w1_small_wait)

        x1 = xf + mod_s[2] * attn
        h2 = _layernorm(x1) * (1.0 + mod_s[4]) + mod_s[3]
        y = _layernorm(h2).astype(bf)
        b1 = b1_v[...].astype(f32).reshape(1, F)
        b2 = b2_v[...].astype(f32).reshape(1, D)
        acc = jnp.broadcast_to(b2, (B, D))
        fc = F // 4
        for i in range(4):
            u = jnp.dot(y, w1_v[:, i * fc:(i + 1) * fc], preferred_element_type=f32) + b1[:, i * fc:(i + 1) * fc]
            a = jax.nn.gelu(u, approximate=True).astype(bf)
            for j in range(6):
                w2_event(i, j).big.wait()
                w2_event(i, j).small.wait()
            acc = acc + jnp.dot(a, w2_v[i * fc:(i + 1) * fc, :], preferred_element_type=f32)
        out_ref[...] = (x1 + mod_s[5] * acc).astype(out_ref.dtype)

    @jax.jit
    def f(A_x, A_k_cache, A_v_cache, A_wq, A_wo, B_x, B_w1, B_b1, B_w2, B_b2, c, w_mod):
        del B_x
        B, Sq, D = A_x.shape
        _, Hkv, SK, Dh = A_k_cache.shape
        W = min(4096, max(256, SK // 4))
        HD = A_wq.shape[1]
        F = B_w1.shape[1]
        NG = Hkv // G
        S = G * Dh // (8 * NB)
        kt = jnp.swapaxes(A_k_cache, 2, 3).reshape(B, NG, NB, S, 8, SK)
        vt = jnp.swapaxes(A_v_cache, 2, 3).reshape(B, NG, NB, S, 8, SK)
        hbm = pl.BlockSpec(memory_space=pltpu.HBM)
        dma = pltpu.SemaphoreType.DMA
        out = pl.pallas_call(
            kernel,
            out_shape=jax.ShapeDtypeStruct((B, D), A_x.dtype),
            in_specs=[hbm] * 11,
            out_specs=pl.BlockSpec(memory_space=pltpu.VMEM),
            scratch_shapes=[
                pltpu.VMEM((B, D), bf), pltpu.VMEM((B, D), bf), pltpu.VMEM((F,), bf), pltpu.VMEM((D,), bf),
                pltpu.VMEM((D, 6 * D), bf), pltpu.VMEM((D, HD), bf), pltpu.VMEM((HD, D), bf),
                pltpu.VMEM((D, F), bf), pltpu.VMEM((F, D), bf),
                pltpu.VMEM((NSLOT, NB, S, 8, W), bf), pltpu.VMEM((NSLOT, NB, S, 8, W), bf),
                pltpu.VMEM((NG * NB, B, S * 8), f32), pltpu.VMEM((NG * NB, B, S * 8), f32),
                pltpu.VMEM((6, B, D), f32),
                dma((4,)), dma((15,)), dma((2, NSLOT)),
            ],
            compiler_params=pltpu.CompilerParams(vmem_limit_bytes=100 * 1024 * 1024,
                                                 disable_bounds_checks=not checks,
                                                 disable_semaphore_checks=not schecks),
        )(A_x.reshape(B, D), kt, vt, A_wq, A_wo, B_w1, B_b1, B_w2, B_b2, c, w_mod)
        return out.reshape(B, Sq, D)

    return f


_impl = make(**dict(CW=1024,checks=True,schecks=True))


@jax.jit
def pallas_adaLN_cond__sliding_block_cached__mixer_channel_mlp__decode_kernel(
    A_x, A_k_cache, A_v_cache, A_wq, A_wo, B_x, B_w1, B_b1, B_w2, B_b2, c, w_mod):
    return _impl(A_x, A_k_cache, A_v_cache, A_wq, A_wo, B_x, B_w1, B_b1, B_w2, B_b2, c, w_mod)
```

```python
import jax
import jax.numpy as jnp
from jax import lax
from jax.experimental import pallas as pl
from jax.experimental.pallas import tpu as pltpu

_EPS = 1e-05
_HEADS = 8
_PARTS = 4
_SLOTS = 3
_PUMPS = 12
_W2_LAST = 384


def _layernorm(x):
    m = jnp.mean(x, axis=-1, keepdims=True)
    d = x - m
    v = jnp.mean(d * d, axis=-1, keepdims=True)
    return d / jnp.sqrt(v + _EPS)


def _kernel(x_hbm, k_hbm, v_hbm, wq_hbm, wo_hbm, w1_hbm, b1_hbm, w2_hbm, b2_hbm, c_hbm, wmod_hbm,
            out_ref,
            x_v, c_v, b1_v, b2_v, wmod_v, wq_v, wo_v, w1_v, w2_v, k_v, v_v, q_s, o_s, mod_s, sem):
    bf16, f32 = jnp.bfloat16, jnp.float32
    B, D = x_v.shape
    F = w2_v.shape[0]
    _, _, S, _, W = k_v.shape
    SK = k_hbm.shape[-1]
    NG = k_hbm.shape[1]
    BR = S * 8
    Dh = BR // 2
    R = wq_v.shape[1]
    nsteps = B * NG
    nit = 2 * _PARTS
    window = pl.ds(SK - W, W)

    def loop(n, body, init=0):
        return lax.fori_loop(0, n, body, init)

    def cols(i, n):
        return pl.ds(pl.multiple_of(i * n, 128), n)

    def spread(i):
        return (i % 4) * (R // 4) + i // 4

    def start_event(src, dst, s):
        head, rest = pl.ds(0, 1), pl.ds(1, _PARTS - 1)
        pltpu.make_async_copy(src.at[head], dst.at[head], s).start(priority=0)
        pltpu.make_async_copy(src.at[rest], dst.at[rest], s).start(priority=1)

    def wait_filled(buf, s):
        pltpu.make_async_copy(buf, buf, s).wait()

    def start_kv(step, it, e):
        slot = step % _SLOTS
        src, dst = ((k_hbm, k_v), (v_hbm, v_v))[e % 2]
        m = e // 2
        u = it * (_PUMPS // 4) + m // 2
        pos = (S // 2) * (m % 2) + (u & ~3) + ((u & 1) << 1) + ((u >> 1) & 1)
        start_event(src.at[step % B, step // B, :, pos, :, window], dst.at[slot, :, pos], sem.at[slot])

    def wait_kv(step):
        slot = step % _SLOTS
        wait_filled(k_v.at[slot], sem.at[slot])
        wait_filled(v_v.at[slot], sem.at[slot])

    s_mod, s_wq = sem.at[2], sem.at[1]
    s_wo, s_w1 = sem.at[nsteps % _SLOTS], sem.at[(nsteps - 2) % _SLOTS]
    s_w2 = (sem.at[(nsteps - 1) % _SLOTS], sem.at[_SLOTS])

    def issue_wmod(i, carry):
        r = spread(i)
        for j in range(3):
            cs = pl.ds(j * 2 * D, 2 * D)
            pltpu.make_async_copy(wmod_hbm.at[:, r, :, cs], wmod_v.at[:, r, :, cs], s_mod).start(priority=1)
        return carry
    loop(R, issue_wmod)
    small = [pltpu.make_async_copy(src, dst, s_mod)
             for src, dst in ((c_hbm, c_v), (x_hbm, x_v), (b1_hbm, b1_v), (b2_hbm, b2_v))]
    for cp in small:
        cp.start()

    def issue_wq(i, carry):
        r = spread(i)
        n = wq_v.shape[-1] // 6
        for j in range(6):
            cs = pl.ds(j * n, n)
            start_event(wq_hbm.at[:, r, :, cs], wq_v.at[:, r, :, cs], s_wq)
        return carry
    loop(R, issue_wq)
    wait_filled(wmod_v, s_mod)
    for cp in small:
        cp.wait()

    cf = c_v[...].astype(f32)
    cond = (cf * jax.nn.sigmoid(cf)).astype(bf16)

    def modulation(it, carry):
        for e in range(_PUMPS):
            start_kv(0, it, e)

        @pl.when(it < 6)
        def _():
            w = wmod_v[:, :, :, cols(it, D)].reshape(D, D)
            mod_s[it] = jnp.dot(cond, w, preferred_element_type=f32)
        return carry
    loop(nit, modulation)
    wait_filled(wq_v, s_wq)

    xf = x_v[...].astype(f32)
    h = (_layernorm(xf) * (1.0 + mod_s[1]) + mod_s[0]).astype(bf16)

    def q_proj(it, carry):
        for half in range(2):
            for e in range(_PUMPS // 2):
                start_kv(1, it, half * (_PUMPS // 2) + e)
            pair = it * 2 + half
            w = wq_v[:, :, :, cols(pair, BR)].reshape(D, BR)
            q_s[pair] = jnp.dot(h, w, preferred_element_type=f32)
        return carry
    loop(nit, q_proj)

    row = lax.broadcasted_iota(jnp.int32, (_HEADS, BR), 0)
    second = (lax.broadcasted_iota(jnp.int32, (_HEADS, BR), 1) >= Dh).astype(jnp.int32)
    per_dot = _PUMPS // (BR // 128)

    def attention(step, pump):
        slot = step % _SLOTS
        b = step % B
        pair0 = (step // B) * _PARTS

        def slab(buf, it, t):
            return buf[slot, it, pl.ds(t * 16, 16)].reshape(128, W)

        def around(it, t, matmul):
            for e in range(per_dot // 2):
                pump(it, t * per_dot + e)
            res = matmul()
            for e in range(per_dot // 2, per_dot):
                pump(it, t * per_dot + e)
            return res

        def qk(it, s):
            own = row == 2 * it + second
            q = jnp.broadcast_to(q_s[pair0 + it, pl.ds(b, 1), :], (_HEADS, BR))
            q = jnp.where(own, q, 0.0).astype(bf16)
            for t in range(BR // 128):
                s = s + around(it, t, lambda: jnp.dot(
                    q[:, t * 128:(t + 1) * 128], slab(k_v, it, t), preferred_element_type=f32))
            return s
        s = loop(_PARTS, qk, jnp.zeros((_HEADS, W), f32)) * Dh ** -0.5
        p = jnp.exp(s - jnp.max(s, axis=-1, keepdims=True))
        inv = 1.0 / jnp.sum(p, axis=-1, keepdims=True)
        p = p.astype(bf16)

        def pv(it, carry):
            o = [around(_PARTS + it, t, lambda: lax.dot_general(
                     p, slab(v_v, it, t), (((1,), (1,)), ((), ())), preferred_element_type=f32))
                 for t in range(BR // 128)]
            o = jnp.where(row == 2 * it + second, jnp.concatenate(o, axis=1) * inv, 0.0)
            o_s[pair0 + it, pl.ds(b, 1), :] = jnp.sum(o, axis=0, keepdims=True)
            return carry
        loop(_PARTS, pv)

    def steady(step, carry):
        wait_kv(step)
        attention(step, lambda it, e: start_kv(step + 2, it, e))
        return carry
    loop(nsteps - 2, steady)

    def issue_wo(it, e):
        j = ((e // 4) * nit + it) * 4 + e % 4
        start_event(wo_hbm.at[:, j], wo_v.at[:, j], s_wo)
    wait_kv(nsteps - 2)
    attention(nsteps - 2, issue_wo)

    def issue_w1(it, e):
        per_it = 2 * R // nit
        if e % 2 == 0 and e // 2 < per_it:
            i = it * per_it + e // 2
            r, cs = spread(i // 2), cols(i % 2, F // 2)
            start_event(w1_hbm.at[:, r, :, cs], w1_v.at[:, r, :, cs], s_w1)
    wait_kv(nsteps - 1)
    attention(nsteps - 1, issue_w1)

    w2_chunks = ((0, F - _W2_LAST), (F - _W2_LAST, _W2_LAST))
    for (r0, n), s in zip(w2_chunks, s_w2):
        for r in range(r0, r0 + n, 64):
            head, rest = pl.ds(r, 16), pl.ds(r + 16, 48)
            pltpu.make_async_copy(w2_hbm.at[head], w2_v.at[head], s).start(priority=0)
            pltpu.make_async_copy(w2_hbm.at[rest], w2_v.at[rest], s).start(priority=1)

    wait_filled(wo_v, s_wo)

    def out_proj(pair, acc):
        n = BR // 16
        w = wo_v[pair // _PARTS, pl.ds((pair % _PARTS) * n, n)].reshape(BR, D)
        return acc + jnp.dot(o_s[pair].astype(bf16), w, preferred_element_type=f32)
    attn = loop(NG * _PARTS, out_proj, jnp.zeros((B, D), f32))
    x1 = xf + mod_s[2] * attn

    h2 = _layernorm(x1) * (1.0 + mod_s[4]) + mod_s[3]
    y = _layernorm(h2).astype(bf16)
    b1 = b1_v[...].astype(f32).reshape(1, F)
    b2 = b2_v[...].astype(f32).reshape(1, D)
    wait_filled(w1_v, s_w1)
    u = jnp.dot(y, w1_v[...].reshape(D, F), preferred_element_type=f32) + b1
    a = jax.nn.gelu(u, approximate=True).astype(bf16)
    mlp = jnp.broadcast_to(b2, (B, D))
    for (r0, n), s in zip(w2_chunks, s_w2):
        wait_filled(w2_v.at[pl.ds(r0, n)], s)
        mlp = mlp + jnp.dot(a[:, r0:r0 + n], w2_v[r0:r0 + n, :], preferred_element_type=f32)
    out_ref[...] = (x1 + mod_s[5] * mlp).astype(out_ref.dtype)


@jax.jit
def pallas_adaLN_cond__sliding_block_cached__mixer_channel_mlp__decode_kernel(
    A_x: jax.Array,
    A_k_cache: jax.Array,
    A_v_cache: jax.Array,
    A_wq: jax.Array,
    A_wo: jax.Array,
    B_x: jax.Array,
    B_w1: jax.Array,
    B_b1: jax.Array,
    B_w2: jax.Array,
    B_b2: jax.Array,
    c: jax.Array,
    w_mod: jax.Array,
):
    del B_x
    B, Sq, D = A_x.shape
    _, Hkv, SK, Dh = A_k_cache.shape
    W = min(4096, max(256, SK // 4))
    HD = A_wq.shape[1]
    F = B_w1.shape[1]
    NG = Hkv // _HEADS
    S = _HEADS * Dh // (8 * _PARTS)
    R = D // (8 * _PARTS)
    assert (Sq, D, Hkv, Dh, HD, F) == (1, 640, 32, 192, 6144, 1536)

    kt = jnp.swapaxes(A_k_cache, 2, 3).reshape(B, NG, _PARTS, S, 8, SK)
    vt = jnp.swapaxes(A_v_cache, 2, 3).reshape(B, NG, _PARTS, S, 8, SK)
    wq = A_wq.reshape(_PARTS, R, 8, HD)
    wo = A_wo.reshape(_PARTS, HD // (16 * _PARTS), 16, D)
    w1 = B_w1.reshape(_PARTS, R, 8, F)
    wmod = w_mod.reshape(_PARTS, R, 8, 6 * D)

    def vmem_like(a):
        return pltpu.VMEM(a.shape, a.dtype)

    x = A_x.reshape(B, D)
    out = pl.pallas_call(
        _kernel,
        out_shape=jax.ShapeDtypeStruct((B, D), A_x.dtype),
        in_specs=[pl.BlockSpec(memory_space=pltpu.HBM)] * 11,
        out_specs=pl.BlockSpec(memory_space=pltpu.VMEM),
        scratch_shapes=[
            vmem_like(x), vmem_like(c), vmem_like(B_b1), vmem_like(B_b2),
            vmem_like(wmod), vmem_like(wq), vmem_like(wo), vmem_like(w1), vmem_like(B_w2),
            pltpu.VMEM((_SLOTS, _PARTS, S, 8, W), kt.dtype),
            pltpu.VMEM((_SLOTS, _PARTS, S, 8, W), vt.dtype),
            pltpu.VMEM((NG * _PARTS, B, S * 8), jnp.float32),
            pltpu.VMEM((NG * _PARTS, B, S * 8), jnp.float32),
            pltpu.VMEM((6, B, D), jnp.float32),
            pltpu.SemaphoreType.DMA((_SLOTS + 1,)),
        ],
        compiler_params=pltpu.CompilerParams(vmem_limit_bytes=64 * 1024 * 1024),
    )(x, kt, vt, wq, wo, w1, B_b1, B_w2, B_b2, c, wmod)
    return out.reshape(B, Sq, D)
```

```python
import jax
import jax.numpy as jnp
from jax import lax
from jax.experimental import pallas as pl
from jax.experimental.pallas import tpu as pltpu

_EPS = 1e-05
_HEADS = 8
_PARTS = 4
_SLOTS = 3
_PUMPS = 12
_W2_LAST = 384


def _layernorm(x):
    m = jnp.mean(x, axis=-1, keepdims=True)
    d = x - m
    v = jnp.mean(d * d, axis=-1, keepdims=True)
    return d / jnp.sqrt(v + _EPS)


def _kernel(x_hbm, k_hbm, v_hbm, wq_hbm, wo_hbm, w1_hbm, b1_hbm, w2_hbm, b2_hbm, c_hbm, wmod_hbm,
            out_ref,
            x_v, c_v, b1_v, b2_v, wmod_v, wq_v, wo_v, w1_v, w2_v, kv_v, q_s, o_s, mod_s, sem):
    bf16, f32 = jnp.bfloat16, jnp.float32
    B, D = x_v.shape
    F = w2_v.shape[0]
    _, _, _, S, _, W = kv_v.shape
    SK = k_hbm.shape[-1]
    NG = k_hbm.shape[1]
    BR = S * 8
    Dh = BR // 2
    R = wq_v.shape[1]
    nsteps = B * NG
    nit = 2 * _PARTS
    window = pl.ds(SK - W, W)

    def loop(n, body, init=0):
        return lax.fori_loop(0, n, body, init)

    def cols(i, n):
        return pl.ds(pl.multiple_of(i * n, 128), n)

    def spread(i):
        return (i % 4) * (R // 4) + i // 4

    def start_event(src, dst, s):
        head, rest = pl.ds(0, 1), pl.ds(1, _PARTS - 1)
        pltpu.make_async_copy(src.at[head], dst.at[head], s).start(priority=0)
        pltpu.make_async_copy(src.at[rest], dst.at[rest], s).start(priority=1)

    def wait_filled(buf, s):
        pltpu.make_async_copy(buf, buf, s).wait()

    def start_kv(step, it, e):
        slot = step % _SLOTS
        src, m = (k_hbm, v_hbm)[e % 2], e // 2
        u = it * (_PUMPS // 4) + m // 2
        pos = (S // 2) * (m % 2) + (u & ~3) + ((u & 1) << 1) + ((u >> 1) & 1)
        start_event(src.at[step % B, step // B, :, pos, :, window], kv_v.at[slot, e % 2, :, pos], sem.at[slot])

    def wait_kv(step):
        slot = step % _SLOTS
        wait_filled(kv_v.at[slot], sem.at[slot])

    s_mod, s_wq = sem.at[2], sem.at[1]
    s_wo, s_w1 = sem.at[nsteps % _SLOTS], sem.at[(nsteps - 2) % _SLOTS]
    s_w2 = (sem.at[(nsteps - 1) % _SLOTS], sem.at[_SLOTS])

    def issue_wmod(i, carry):
        r = spread(i)
        for j in range(3):
            cs = pl.ds(j * 2 * D, 2 * D)
            pltpu.make_async_copy(wmod_hbm.at[:, r, :, cs], wmod_v.at[:, r, :, cs], s_mod).start(priority=1)
        return carry
    loop(R, issue_wmod)
    small = [pltpu.make_async_copy(src, dst, sem.at[_SLOTS])
             for src, dst in ((c_hbm, c_v), (x_hbm, x_v), (b1_hbm, b1_v), (b2_hbm, b2_v))]
    for cp in small:
        cp.start()

    def issue_wq(i, carry):
        r = spread(i)
        n = wq_v.shape[-1] // 6
        for j in range(6):
            cs = pl.ds(j * n, n)
            start_event(wq_hbm.at[:, r, :, cs], wq_v.at[:, r, :, cs], s_wq)
        return carry
    loop(R, issue_wq)
    wait_filled(wmod_v, s_mod)
    for cp in small:
        cp.wait()

    cf = c_v[...].astype(f32)
    cond = (cf * jax.nn.sigmoid(cf)).astype(bf16)

    def modulation(it, carry):
        for e in range(_PUMPS):
            start_kv(0, it, e)

        @pl.when(it < 6)
        def _():
            w = wmod_v[:, :, :, cols(it, D)].reshape(D, D)
            mod_s[it] = jnp.dot(cond, w, preferred_element_type=f32)
        return carry
    loop(nit, modulation)
    wait_filled(wq_v, s_wq)

    xf = x_v[...].astype(f32)
    h = (_layernorm(xf) * (1.0 + mod_s[1]) + mod_s[0]).astype(bf16)

    def q_proj(it, carry):
        for half in range(2):
            for e in range(_PUMPS // 2):
                start_kv(1, it, half * (_PUMPS // 2) + e)
            pair = it * 2 + half
            w = wq_v[:, :, :, cols(pair, BR)].reshape(D, BR)
            q_s[pair] = jnp.dot(h, w, preferred_element_type=f32)
        return carry
    loop(nit, q_proj)

    row = lax.broadcasted_iota(jnp.int32, (_HEADS, BR), 0)
    second = (lax.broadcasted_iota(jnp.int32, (_HEADS, BR), 1) >= Dh).astype(jnp.int32)
    per_dot = _PUMPS // (BR // 128)

    def attention(step, pump):
        slot = step % _SLOTS
        b = step % B
        pair0 = (step // B) * _PARTS

        def slab(which, it, t):
            return kv_v[slot, which, it, pl.ds(t * 16, 16)].reshape(128, W)

        def around(it, t, matmul):
            for e in range(per_dot // 2):
                pump(it, t * per_dot + e)
            res = matmul()
            for e in range(per_dot // 2, per_dot):
                pump(it, t * per_dot + e)
            return res

        def qk(it, s):
            own = row == 2 * it + second
            q = jnp.broadcast_to(q_s[pair0 + it, pl.ds(b, 1), :], (_HEADS, BR))
            q = jnp.where(own, q, 0.0).astype(bf16)
            for t in range(BR // 128):
                s = s + around(it, t, lambda: jnp.dot(
                    q[:, t * 128:(t + 1) * 128], slab(0, it, t), preferred_element_type=f32))
            return s
        s = loop(_PARTS, qk, jnp.zeros((_HEADS, W), f32)) * Dh ** -0.5
        p = jnp.exp(s - jnp.max(s, axis=-1, keepdims=True))
        inv = 1.0 / jnp.sum(p, axis=-1, keepdims=True)
        p = p.astype(bf16)

        def pv(it, carry):
            o = [around(_PARTS + it, t, lambda: lax.dot_general(
                     p, slab(1, it, t), (((1,), (1,)), ((), ())), preferred_element_type=f32))
                 for t in range(BR // 128)]
            o = jnp.where(row == 2 * it + second, jnp.concatenate(o, axis=1) * inv, 0.0)
            o_s[pair0 + it, pl.ds(b, 1), :] = jnp.sum(o, axis=0, keepdims=True)
            return carry
        loop(_PARTS, pv)

    def steady(step, carry):
        wait_kv(step)
        attention(step, lambda it, e: start_kv(step + 2, it, e))
        return carry
    loop(nsteps - 2, steady)

    def issue_wo(it, e):
        j = ((e // 4) * nit + it) * 4 + e % 4
        start_event(wo_hbm.at[:, j], wo_v.at[:, j], s_wo)
    wait_kv(nsteps - 2)
    attention(nsteps - 2, issue_wo)

    def issue_w1(it, e):
        per_it = 2 * R // nit
        if e % 2 == 0 and e // 2 < per_it:
            i = it * per_it + e // 2
            r, cs = spread(i // 2), cols(i % 2, F // 2)
            start_event(w1_hbm.at[:, r, :, cs], w1_v.at[:, r, :, cs], s_w1)
    wait_kv(nsteps - 1)
    attention(nsteps - 1, issue_w1)

    w2_chunks = ((0, F - _W2_LAST), (F - _W2_LAST, _W2_LAST))
    for (r0, n), s in zip(w2_chunks, s_w2):
        for r in range(r0, r0 + n, 64):
            head, rest = pl.ds(r, 16), pl.ds(r + 16, 48)
            pltpu.make_async_copy(w2_hbm.at[head], w2_v.at[head], s).start(priority=0)
            pltpu.make_async_copy(w2_hbm.at[rest], w2_v.at[rest], s).start(priority=1)

    wait_filled(wo_v, s_wo)

    def out_proj(pair, acc):
        n = BR // 16
        w = wo_v[pair // _PARTS, pl.ds((pair % _PARTS) * n, n)].reshape(BR, D)
        return acc + jnp.dot(o_s[pair].astype(bf16), w, preferred_element_type=f32)
    attn = loop(NG * _PARTS, out_proj, jnp.zeros((B, D), f32))
    x1 = xf + mod_s[2] * attn

    h2 = _layernorm(x1) * (1.0 + mod_s[4]) + mod_s[3]
    y = _layernorm(h2).astype(bf16)
    b1 = b1_v[...].astype(f32).reshape(1, F)
    b2 = b2_v[...].astype(f32).reshape(1, D)
    wait_filled(w1_v, s_w1)
    u = jnp.dot(y, w1_v[...].reshape(D, F), preferred_element_type=f32) + b1
    a = jax.nn.gelu(u, approximate=True).astype(bf16)
    mlp = jnp.broadcast_to(b2, (B, D))
    for (r0, n), s in zip(w2_chunks, s_w2):
        wait_filled(w2_v.at[pl.ds(r0, n)], s)
        mlp = mlp + jnp.dot(a[:, r0:r0 + n], w2_v[r0:r0 + n, :], preferred_element_type=f32)
    out_ref[...] = (x1 + mod_s[5] * mlp).astype(out_ref.dtype)


@jax.jit
def pallas_adaLN_cond__sliding_block_cached__mixer_channel_mlp__decode_kernel(
    A_x: jax.Array,
    A_k_cache: jax.Array,
    A_v_cache: jax.Array,
    A_wq: jax.Array,
    A_wo: jax.Array,
    B_x: jax.Array,
    B_w1: jax.Array,
    B_b1: jax.Array,
    B_w2: jax.Array,
    B_b2: jax.Array,
    c: jax.Array,
    w_mod: jax.Array,
):
    del B_x
    B, Sq, D = A_x.shape
    _, Hkv, SK, Dh = A_k_cache.shape
    W = min(4096, max(256, SK // 4))
    HD = A_wq.shape[1]
    F = B_w1.shape[1]
    NG = Hkv // _HEADS
    S = _HEADS * Dh // (8 * _PARTS)
    R = D // (8 * _PARTS)
    assert (Sq, D, Hkv, Dh, HD, F) == (1, 640, 32, 192, 6144, 1536)

    kt = jnp.swapaxes(A_k_cache, 2, 3).reshape(B, NG, _PARTS, S, 8, SK)
    vt = jnp.swapaxes(A_v_cache, 2, 3).reshape(B, NG, _PARTS, S, 8, SK)
    wq = A_wq.reshape(_PARTS, R, 8, HD)
    wo = A_wo.reshape(_PARTS, HD // (16 * _PARTS), 16, D)
    w1 = B_w1.reshape(_PARTS, R, 8, F)
    wmod = w_mod.reshape(_PARTS, R, 8, 6 * D)

    def vmem_like(a):
        return pltpu.VMEM(a.shape, a.dtype)

    x = A_x.reshape(B, D)
    out = pl.pallas_call(
        _kernel,
        out_shape=jax.ShapeDtypeStruct((B, D), A_x.dtype),
        in_specs=[pl.BlockSpec(memory_space=pltpu.HBM)] * 11,
        out_specs=pl.BlockSpec(memory_space=pltpu.VMEM),
        scratch_shapes=[
            vmem_like(x), vmem_like(c), vmem_like(B_b1), vmem_like(B_b2),
            vmem_like(wmod), vmem_like(wq), vmem_like(wo), vmem_like(w1), vmem_like(B_w2),
            pltpu.VMEM((_SLOTS, 2, _PARTS, S, 8, W), kt.dtype),
            pltpu.VMEM((NG * _PARTS, B, S * 8), jnp.float32),
            pltpu.VMEM((NG * _PARTS, B, S * 8), jnp.float32),
            pltpu.VMEM((6, B, D), jnp.float32),
            pltpu.SemaphoreType.DMA((_SLOTS + 1,)),
        ],
        compiler_params=pltpu.CompilerParams(vmem_limit_bytes=64 * 1024 * 1024),
    )(x, kt, vt, wq, wo, w1, B_b1, B_w2, B_b2, c, wmod)
    return out.reshape(B, Sq, D)
```
